```python
import jax
import jax.numpy as jnp

def _softmax(x, axis=-1):
    return jax.nn.softmax(x, axis=axis)

def _gelu(x):
    return jax.nn.gelu(x, approximate=True)

def _silu(x):
    return jax.nn.silu(x)

def _sigmoid(x):
    return jax.nn.sigmoid(x)

def _layernorm(x, axis=-1, eps=1e-05):
    m = jnp.mean(x, axis=axis, keepdims=True)
    v = jnp.var(x, axis=axis, keepdims=True)
    return (x - m) / jnp.sqrt(v + eps)

def _scatter_add(tgt, idx, src, axis=0):
    return tgt.at[idx].add(src)

def _segment_sum(src, seg, n):
    return jax.ops.segment_sum(src, seg, n)

class _Rng:

    def __init__(self, key):
        self._k = key

    def _next(self):
        self._k, sub = jax.random.split(self._k)
        return sub

    def normal(self, shape):
        return jax.random.normal(self._next(), shape, dtype=jnp.bfloat16)

    def randint(self, lo, hi, shape):
        return jax.random.randint(self._next(), shape, lo, hi, dtype=jnp.int32)

    def uniform(self, shape, lo=0.0, hi=1.0):
        return jax.random.uniform(self._next(), shape, jnp.bfloat16, lo, hi)

    def permutation(self, n):
        return jax.random.permutation(self._next(), n)
kernel_name = 'recurrent_scan__memory_aug_recurrent_mem_tr__mixer_s_mlp__prompt'

def setup_inputs():
    _rng = _Rng(jax.random.key(int.from_bytes(__import__("os").urandom(4), "little")))
    _w = lambda a: (lambda t: t.astype(jnp.bfloat16) if jnp.issubdtype(t.dtype, jnp.floating) else t)(jnp.asarray(a))

    def _A_setup():
        B, S, Dm = (1, 2048, 1024)
        H, Dh = (32, 128)
        M, seg = (8, 32)
        seg = min(seg, S)
        S = S // seg * seg
        return {'x': _w((lambda *s: _rng.normal(s) * 0.05)(B, S, Dm)), 'mem0': _w((lambda *s: _rng.normal(s) * 0.05)(B, M, Dm)), 'Wq': _w((lambda *s: _rng.normal(s) * 0.05)(Dm, H, Dh) * Dm ** (-0.5)), 'Wk': _w((lambda *s: _rng.normal(s) * 0.05)(Dm, H, Dh) * Dm ** (-0.5)), 'Wv': _w((lambda *s: _rng.normal(s) * 0.05)(Dm, H, Dh) * Dm ** (-0.5)), 'Wo': _w((lambda *s: _rng.normal(s) * 0.05)(H, Dh, Dm) * (H * Dh) ** (-0.5)), 'seg_len': seg}
    _A_in = _A_setup()

    def _B_setup():
        B, S, D, F = (1, 2048, 1024, 3584)
        return {'x': _w((lambda *s: _rng.normal(s) * 0.05)(B, S, D)), 'w1': _w((lambda *s: _rng.normal(s) * 0.05)(D, D) * D ** (-0.5)), 'w2': _w((lambda *s: _rng.normal(s) * 0.05)(D, D) * D ** (-0.5)), 'w3': _w((lambda *s: _rng.normal(s) * 0.05)(D, F) * D ** (-0.5)), 'w4': _w((lambda *s: _rng.normal(s) * 0.05)(F, D) * F ** (-0.5))}
    _B_in = _B_setup()
    return {'A_x': _A_in['x'], 'A_mem0': _A_in['mem0'], 'A_Wq': _A_in['Wq'], 'A_Wk': _A_in['Wk'], 'A_Wv': _A_in['Wv'], 'A_Wo': _A_in['Wo'], 'A_seg_len': _A_in['seg_len'], 'B_x': _B_in['x'], 'B_w1': _B_in['w1'], 'B_w2': _B_in['w2'], 'B_w3': _B_in['w3'], 'B_w4': _B_in['w4']}

def reference(A_x, A_mem0, A_Wq, A_Wk, A_Wv, A_Wo, A_seg_len, B_x, B_w1, B_w2, B_w3, B_w4):

    def _A_ref(x, mem0, Wq, Wk, Wv, Wo, seg_len):
        B, S, Dm = x.shape
        H, Dh = (Wq.shape[1], Wq.shape[2])
        M = mem0.shape[1]
        scale = Dh ** (-0.5)
        n_seg = S // seg_len
        L = M + seg_len
        idx = jnp.arange(L)
        mask = (idx[:, None] < M) | (idx[:, None] >= idx[None, :])
        mem = mem0
        outs = []
        for s in range(n_seg):
            xs = x[:, s * seg_len:(s + 1) * seg_len, :].copy()
            h = jnp.concatenate([mem, xs], axis=1)
            q = jnp.einsum('btd,dhe->bhte', h, Wq)
            k = jnp.einsum('btd,dhe->bhte', h, Wk)
            v = jnp.einsum('btd,dhe->bhte', h, Wv)
            scores = jnp.einsum('bhqe,bhke->bhqk', q, k) * scale
            scores = jnp.where(mask[None, None], scores, -1000000000.0)
            p = _softmax(scores, axis=-1)
            o = jnp.einsum('bhqk,bhke->bhqe', p, v)
            o = jnp.einsum('bhte,hed->btd', o, Wo)
            mem = o[:, :M, :].copy()
            outs.append(o[:, M:, :])
        return jnp.concatenate(outs, axis=1)

    def _B_ref(x, w1, w2, w3, w4):
        B, S, D = x.shape
        h = _gelu(_layernorm(x, axis=-1) @ w1)
        c = D // 4
        g0 = jnp.pad(h[:, :, 0 * c:1 * c], ((0, 0), (1, 0), (0, 0)))[:, :S, :]
        g1 = jnp.pad(h[:, :, 1 * c:2 * c], ((0, 0), (0, 1), (0, 0)))[:, 1:, :]
        g2 = jnp.pad(h[:, :, 2 * c:3 * c], ((0, 0), (2, 0), (0, 0)))[:, :S, :]
        g3 = jnp.pad(h[:, :, 3 * c:], ((0, 0), (0, 2), (0, 0)))[:, 2:, :]
        hs = jnp.concatenate([g0, g1, g2, g3], axis=-1) @ w2
        x1 = x + hs
        h2 = _gelu(_layernorm(x1, axis=-1) @ w3) @ w4
        return x1 + h2
    x = A_x
    xn = _layernorm(x, axis=-1)
    s = _A_ref(xn, A_mem0, A_Wq, A_Wk, A_Wv, A_Wo, A_seg_len)
    g = _silu(_B_ref(xn, B_w1, B_w2, B_w3, B_w4))
    return x + s * g
```

```python
import functools

import jax
import jax.numpy as jnp
import numpy as np
from jax import lax
from jax.experimental import pallas as pl
from jax.experimental.pallas import tpu as pltpu

F32 = jnp.float32
BF16 = jnp.bfloat16
U32 = jnp.uint32
_LO = np.uint32(0x0000FFFF)
_HI = np.uint32(0xFFFF0000)
_EPS = 1e-5
_HALO = 8


def _mm(a, b):
    return lax.dot_general(a, b, (((1,), (0,)), ((), ())), preferred_element_type=F32)


def _mm_nt(a, b):
    return lax.dot_general(a, b, (((1,), (1,)), ((), ())), preferred_element_type=F32)


def _w(u):
    return pltpu.bitcast(u, BF16)


def _layernorm(x):
    m = jnp.mean(x, axis=-1, keepdims=True)
    d = x - m
    v = jnp.mean(d * d, axis=-1, keepdims=True)
    return d * lax.rsqrt(v + _EPS)


def _gelu(x):
    c = float(np.sqrt(2.0 / np.pi))
    t = jnp.tanh(x * (c + (c * 0.044715) * (x * x)))
    hx = 0.5 * x
    return hx + hx * t


def _silu(x):
    return x / (1.0 + jnp.exp(-x))


def _kernel(x_hbm, mem0_ref, wq_hbm, wk_hbm, wv_hbm, wo_hbm, w1_hbm, w2_hbm, w3_hbm, w4_hbm,
            o_hbm,
            x_v, xn_v, hb_v, g_v, wq_v, wk_v, wv_v, wo_v, w1_v, w2_v, w3_v, w4_v, h_v, ob_v,
            sem_x, sem_w, sem_a, sem_o,
            *, S, D, F, H, Dh, M, SEG, R, FC):
    nblk = S // R
    nseg = S // SEG
    L = M + SEG
    HP = H // 2

    def x_copy(i):
        r = pl.ds(pl.multiple_of(i * R, R), R)
        return pltpu.make_async_copy(x_hbm.at[r, :], x_v.at[r, :], sem_x.at[i])

    w_copies = [
        pltpu.make_async_copy(src.bitcast(U32), dst, sem_w.at[n])
        for n, (src, dst) in enumerate(
            [(w1_hbm, w1_v), (w2_hbm, w2_v), (w3_hbm, w3_v), (w4_hbm, w4_v), (wo_hbm, wo_v)])
    ]

    def qkv_copies(n, src, dst):
        su = src.bitcast(U32)
        return [pltpu.make_async_copy(su.at[:, p, j, :], dst.at[j, p], sem_a.at[n])
                for j in range(HP) for p in range(2)]

    a_copies = [qkv_copies(n, s_, d_)
                for n, (s_, d_) in enumerate([(wq_hbm, wq_v), (wk_hbm, wk_v), (wv_hbm, wv_v)])]

    x_copy(0).start()
    w_copies[0].start()
    zeros = jnp.zeros((_HALO, D), F32)
    hb_v[0:_HALO, :] = zeros
    hb_v[_HALO + S:, :] = zeros
    w_copies[0].wait()
    for i in range(1, nblk):
        x_copy(i).start()
    for c in w_copies[1:4]:
        c.start()

    def stage1(i, _):
        r0 = pl.multiple_of(i * R, R)
        x_copy(i).wait()
        xn = _layernorm(x_v[pl.ds(r0, R), :].astype(F32)).astype(BF16)
        xn_v[pl.ds(r0, R), :] = xn
        xnn = _layernorm(xn.astype(F32)).astype(BF16)
        hb_v[pl.ds(r0 + _HALO, R), :] = _gelu(_mm(xnn, _w(w1_v[...])))
        return 0

    lax.fori_loop(0, nblk, stage1, 0)

    for c in w_copies[1:4]:
        c.wait()
    for cs in a_copies:
        for c in cs:
            c.start()
    w_copies[4].start()

    def stage2(i, _):
        r0 = pl.multiple_of(i * R, R)
        c = D // 4
        parts = []
        for j, sh in enumerate((-1, 1, -2, 2)):
            win = hb_v[pl.ds(r0, R + 2 * _HALO), j * c:(j + 1) * c]
            parts.append(win[_HALO + sh:_HALO + sh + R])
        hs = _mm(jnp.concatenate(parts, axis=1).astype(BF16), _w(w2_v[...]))
        x1 = xn_v[pl.ds(r0, R), :].astype(F32) + hs
        l = _layernorm(x1).astype(BF16)
        acc = x1
        for f0 in range(0, F, FC):
            u = _gelu(_mm(l, _w(w3_v[:, f0:f0 + FC]))).astype(BF16)
            acc = acc + _mm(u, _w(w4_v[f0 // 2:(f0 + FC) // 2, :]))
        g_v[pl.ds(r0, R), :] = _silu(acc)
        return 0

    lax.fori_loop(0, nblk, stage2, 0)

    for cs in a_copies:
        for c in cs:
            c.wait()
    w_copies[4].wait()

    def repack(j, _):
        for w in (wq_v, wk_v, wv_v):
            a = w[j, 0]
            b = w[j, 1]
            w[j, 0] = (a & _LO) | (b << 16)
            w[j, 1] = (a >> 16) | (b & _HI)
        return 0

    lax.fori_loop(0, HP, repack, 0)

    h_v[0:M, :] = mem0_ref[...].astype(F32)
    row = lax.broadcasted_iota(jnp.int32, (L, L), 0)
    col = lax.broadcasted_iota(jnp.int32, (L, L), 1)
    mask = (row < M) | (row >= col)
    scale = Dh ** -0.5
    osplit = H - 4

    def step(s, _):
        r0 = pl.multiple_of(s * SEG, SEG)
        h_v[M:L, :] = xn_v[pl.ds(r0, SEG), :].astype(F32)

        def proj(h):
            w = jnp.concatenate([wq_v[h // 2, h % 2], wk_v[h // 2, h % 2], wv_v[h // 2, h % 2]], axis=1)
            return _mm(h_v[...], _w(w))

        def scores(qkv):
            return _mm_nt(qkv[:, 0:Dh], qkv[:, Dh:2 * Dh])

        def attend(h, qkv, sc):
            sc = jnp.where(mask, sc * scale, -1e9)
            p = jnp.exp(sc - jnp.max(sc, axis=-1, keepdims=True))
            den = jnp.sum(p, axis=-1, keepdims=True)
            ob_v[:, h * Dh:(h + 1) * Dh] = _mm(p, qkv[:, 2 * Dh:]) * (1.0 / den)

        def oproj(h0, h1):
            return _mm(ob_v[:, h0 * Dh:h1 * Dh], _w(wo_v[h0 * Dh // 2:h1 * Dh // 2, :]))

        qkv, sc, acc = {}, {}, None
        for t in range(H + 2):
            if t < H:
                qkv[t] = proj(t)
            elif t == H:
                acc = oproj(0, osplit // 2)
            else:
                acc = acc + oproj(osplit // 2, osplit)
            if 0 <= t - 2 < H:
                attend(t - 2, qkv.pop(t - 2), sc.pop(t - 2))
            if 0 <= t - 1 < H:
                sc[t - 1] = scores(qkv[t - 1])
        acc = acc + oproj(osplit, H)
        h_v[0:M, :] = acc[0:M]
        rows = pl.ds(r0, SEG)
        x_v[rows, :] = (x_v[rows, :].astype(F32) + acc[M:] * g_v[rows, :]).astype(BF16)
        pltpu.make_async_copy(x_v.at[rows, :], o_hbm.at[rows, :], sem_o.at[0]).start()
        return 0

    lax.fori_loop(0, nseg, step, 0)
    pltpu.make_async_copy(x_v, o_hbm, sem_o.at[0]).wait()


@functools.partial(jax.jit, static_argnames=("A_seg_len",))
def pallas_recurrent_scan__memory_aug_recurrent_mem_tr__mixer_s_mlp__prompt_kernel(
    A_x: jax.Array,
    A_mem0: jax.Array,
    A_Wq: jax.Array,
    A_Wk: jax.Array,
    A_Wv: jax.Array,
    A_Wo: jax.Array,
    A_seg_len: int,
    B_x: jax.Array,
    B_w1: jax.Array,
    B_w2: jax.Array,
    B_w3: jax.Array,
    B_w4: jax.Array,
):
    del B_x
    B, S, D = A_x.shape
    assert B == 1
    _, H, Dh = A_Wq.shape
    M = A_mem0.shape[1]
    F = B_w3.shape[1]
    SEG = int(A_seg_len)
    L = M + SEG
    R, FC = 256, 512
    assert S % R == 0 and S % SEG == 0 and F % FC == 0 and H % 2 == 0

    kern = functools.partial(_kernel, S=S, D=D, F=F, H=H, Dh=Dh, M=M, SEG=SEG, R=R, FC=FC)
    hbm = pl.BlockSpec(memory_space=pl.ANY)
    qkv_shape = (D // 2, 2, H, Dh)
    out = pl.pallas_call(
        kern,
        out_shape=jax.ShapeDtypeStruct((S, D), BF16),
        in_specs=[hbm, pl.BlockSpec(memory_space=pltpu.VMEM)] + [hbm] * 8,
        out_specs=hbm,
        scratch_shapes=[
            pltpu.VMEM((S, D), BF16),
            pltpu.VMEM((S, D), BF16),
            pltpu.VMEM((S + 2 * _HALO, D), F32),
            pltpu.VMEM((S, D), F32),
            pltpu.VMEM((H // 2, 2, D // 2, Dh), U32),
            pltpu.VMEM((H // 2, 2, D // 2, Dh), U32),
            pltpu.VMEM((H // 2, 2, D // 2, Dh), U32),
            pltpu.VMEM((H * Dh // 2, D), U32),
            pltpu.VMEM((D // 2, D), U32),
            pltpu.VMEM((D // 2, D), U32),
            pltpu.VMEM((D // 2, F), U32),
            pltpu.VMEM((F // 2, D), U32),
            pltpu.VMEM((L, D), F32),
            pltpu.VMEM((L, H * Dh), F32),
            pltpu.SemaphoreType.DMA((S // R,)),
            pltpu.SemaphoreType.DMA((5,)),
            pltpu.SemaphoreType.DMA((3,)),
            pltpu.SemaphoreType.DMA((1,)),
        ],
        compiler_params=pltpu.CompilerParams(vmem_limit_bytes=110 * 1024 * 1024),
        name="rmt_mixer",
    )(
        A_x.reshape(S, D),
        A_mem0.reshape(M, D),
        A_Wq.reshape(qkv_shape),
        A_Wk.reshape(qkv_shape),
        A_Wv.reshape(qkv_shape),
        A_Wo.reshape(H * Dh, D),
        B_w1, B_w2, B_w3, B_w4,
    )
    return out.reshape(B, S, D)
```

```python
import functools

import jax
import jax.numpy as jnp
import numpy as np
from jax import lax
from jax.experimental import pallas as pl
from jax.experimental.pallas import tpu as pltpu

F32 = jnp.float32
BF16 = jnp.bfloat16
U32 = jnp.uint32
_LO = np.uint32(0x0000FFFF)
_HI = np.uint32(0xFFFF0000)
_EPS = 1e-5
_HALO = 8
_SB = 128
_FC = 512
_NC = 4
_MIX_UNROLL = 2
_SCAN_UNROLL = 2


def _mm(a, b):
    return lax.dot_general(a, b, (((1,), (0,)), ((), ())), preferred_element_type=F32)


def _mm_nt(a, b):
    return lax.dot_general(a, b, (((1,), (1,)), ((), ())), preferred_element_type=F32)


def _w(u):
    return pltpu.bitcast(u, BF16)


def _layernorm(x):
    m = jnp.mean(x, axis=-1, keepdims=True)
    d = x - m
    v = jnp.mean(d * d, axis=-1, keepdims=True)
    return d * lax.rsqrt(v + _EPS)


def _gelu(x):
    c = float(np.sqrt(2.0 / np.pi))
    t = jnp.tanh(x * (c + (c * 0.044715) * (x * x)))
    hx = 0.5 * x
    return hx + hx * t


def _silu(x):
    hx = 0.5 * x
    return hx + hx * jnp.tanh(hx)


def _strassen_lhs(a11, a12, a21, a22):
    ops = (a11 + a22, a21 + a22, a11, a22, a11 + a12, a21 - a11, a12 - a22)
    return [o.astype(BF16) for o in ops]


def _strassen_rhs(w_v, t_v, c, n):
    kh, nh = w_v.shape[1] // 2, w_v.shape[2] // 2
    if n == 1:
        return _w(w_v[c, :kh, :nh])
    if n == 4:
        return _w(w_v[c, kh:, nh:])
    return _w(t_v[c, {0: 0, 2: 1, 3: 2, 5: 3, 6: 4}[n]])


def _strassen_out(m):
    top = jnp.concatenate([m[0] + m[3] - m[4] + m[6], m[2] + m[4]], axis=1)
    bot = jnp.concatenate([m[1] + m[3], m[0] - m[1] + m[2] + m[5]], axis=1)
    return top, bot


def _presum_jobs(w_v, t_v, c):
    kh, nh = w_v.shape[1] // 2, w_v.shape[2] // 2

    def job(r, l):
        def run(zero):
            def quad(i, j):
                u = w_v[c, i * kh + r:i * kh + r + 8, j * nh + l:j * nh + l + 128]
                return _w(u if zero is None else u | zero).astype(F32)
            b11, b12, b21, b22 = quad(0, 0), quad(0, 1), quad(1, 0), quad(1, 1)
            for n, t in enumerate((b11 + b22, b12 - b22, b21 - b11, b11 + b12, b21 + b22)):
                t_v[c, n, r:r + 8, l:l + 128] = pltpu.bitcast(t.astype(BF16), U32)
        return run

    return [job(r, l) for r in range(0, kh, 8) for l in range(0, nh, 128)]


def _spread(jobs, n, after):
    tiles = [(r, c) for c in range(0, after.shape[1], 128) for r in range(0, after.shape[0], 8)]
    n = min(n, len(jobs))
    for k in range(n):
        r, c = tiles[k * len(tiles) // n]
        zero = lax.population_count(pltpu.bitcast(after[r:r + 8, c:c + 128], U32)) >> 6
        jobs.pop(0)(zero)


def _kernel(x_hbm, mem0_hbm, wq_hbm, wk_hbm, wv_hbm, wo_hbm, w1_hbm, w2_hbm, w3_hbm, w4_hbm,
            o_hbm,
            x_v, mem0_v, xn_v, p_v, hb_v, g_v, la_v,
            wqkv_v, wo_v, w1_v, w2_v, w3_v, w4_v, t2_v, t3_v, t4_v,
            sem_w, sem_m, sem_a, sem_o,
            *, S, D, F, H, Dh, M, SEG):
    SB, FC, NC = _SB, _FC, _NC
    R = 2 * SB
    nblk = S // R
    nsb = S // SB
    nch = F // FC
    L = M + SEG
    PPI = H // 2 // nblk
    CW = D // NC

    sems = iter(range(sem_w.shape[0]))

    def copy(src, dst):
        return pltpu.make_async_copy(src, dst, sem_w.at[next(sems)])

    x_copies = [copy(x_hbm.at[lo * SB:hi * SB, :], x_v.at[lo * SB:hi * SB, :])
                for lo, hi in ((0, 2), (2, 3), (3, 5), (5, 7), (7, nsb))]
    w1u, w3u, w4u = w1_hbm.bitcast(U32), w3_hbm.bitcast(U32), w4_hbm.bitcast(U32)
    w1_copies = [copy(w1u.at[:, c * CW:(c + 1) * CW], w1_v.at[:, c * CW:(c + 1) * CW])
                 for c in range(NC)]
    w2_copy = copy(w2_hbm.bitcast(U32), w2_v.at[0])
    a_copies = [copy(mem0_hbm, mem0_v), copy(wo_hbm.bitcast(U32), wo_v)]

    def mlp_copies(c):
        return [pltpu.make_async_copy(w3u.at[:, pl.ds(c * FC, FC)], w3_v.at[c], sem_m.at[c]),
                pltpu.make_async_copy(w4u.at[pl.ds(c * (FC // 2), FC // 2), :], w4_v.at[c],
                                      sem_m.at[nch + c])]

    def qkv_start(i):
        for n, src in enumerate((wq_hbm, wk_hbm, wv_hbm)):
            for j in range(PPI):
                for p in range(2):
                    pltpu.make_async_copy(src.bitcast(U32).at[:, p, i * PPI + j, :],
                                          wqkv_v.at[i * PPI + j, n, p], sem_a.at[i]).start()

    def qkv_wait(i):
        dst = wqkv_v.at[pl.ds(i * PPI, PPI)]
        pltpu.make_async_copy(dst, dst, sem_a.at[i]).wait()

    for c in (x_copies[:1] + w1_copies[:-1] + x_copies[1:2] + w1_copies[-1:] + x_copies[2:]
              + [w2_copy]):
        c.start()
    for c in range(nch):
        for cp in mlp_copies(c):
            cp.start()

    zeros = jnp.zeros((_HALO, D), F32)
    hb_v[0:_HALO, :] = zeros
    hb_v[_HALO + S:, :] = zeros

    def norm(r0):
        xn = _layernorm(x_v[pl.ds(r0, SB), :].astype(F32)).astype(BF16).astype(F32)
        xn_v[pl.ds(r0, SB), :] = xn
        return _layernorm(xn).astype(BF16)

    def hidden(r0, xnn, c0, c1):
        hb_v[pl.ds(r0 + _HALO, SB), c0:c1] = _gelu(_mm(xnn, _w(w1_v[:, c0:c1])))

    x_copies[0].wait()
    xnn = [norm(0), norm(SB)]
    for n in range(NC):
        if n == NC - 1:
            x_copies[1].wait()
        w1_copies[n].wait()
        for b in range(2):
            hidden(b * SB, xnn[b], n * CW, (n + 1) * CW)
    p_v[...] = norm(2 * SB)

    @pl.loop(1, nsb // 2)
    def _(i):
        for k in range(1, 4):
            @pl.when(i == k)
            def _():
                x_copies[k + 1].wait()
        r0 = pl.multiple_of(2 * i * SB, SB)
        hidden(r0, p_v[...], 0, D)
        hidden(r0 + SB, norm(r0 + SB), 0, D)
        p_v[...] = norm(pl.multiple_of(jnp.minimum(r0 + 2 * SB, S - SB), SB))

    w2_copy.wait()
    qkv_start(0)
    qkv_start(1)
    for job in _presum_jobs(w2_v, t2_v, 0):
        job(None)

    def shifted(r0):
        q = D // 4
        parts = []
        for j, sh in enumerate((-1, 1, -2, 2)):
            win = hb_v[pl.ds(r0, SB + 2 * _HALO), j * q:(j + 1) * q]
            parts.append(win[_HALO + sh:_HALO + sh + SB])
        return jnp.concatenate(parts, axis=1)

    @pl.loop(0, nblk // _MIX_UNROLL)
    def _(it):
        blocks = [it * _MIX_UNROLL + u for u in range(_MIX_UNROLL)]
        for i in blocks:
            @pl.when(i < nch)
            def _():
                for cp in mlp_copies(i):
                    cp.wait()
        jobs = []
        for i in blocks:
            c = jnp.minimum(i, nch - 1)
            jobs += _presum_jobs(w3_v, t3_v, c) + _presum_jobs(w4_v, t4_v, c)
        per = -(-len(jobs) // (7 * _MIX_UNROLL))
        for i in blocks:
            r0 = [pl.multiple_of(i * R + b * SB, SB) for b in range(2)]
            ha, hb = shifted(r0[0]), shifted(r0[1])
            lhs = _strassen_lhs(ha[:, :D // 2], ha[:, D // 2:], hb[:, :D // 2], hb[:, D // 2:])
            m = [None] * 7
            for n in (2, 4, 3, 0, 6, 1, 5):
                m[n] = _mm(lhs[n], _strassen_rhs(w2_v, t2_v, 0, n))
                _spread(jobs, per, m[n])
            hs = _strassen_out(m)
            xs = [xn_v[pl.ds(r, SB), :] for r in r0]
            for b in range(2):
                x1 = xs[b] + hs[b]
                g_v[pl.ds(r0[b], SB), :] = x1
                if b == 0:
                    la_v[pl.ds(pl.multiple_of(i * SB, SB), SB), :] = _layernorm(x1)
        assert not jobs

    for c in a_copies:
        c.start()
    order = (2, 4, 3, 1, 0, 5, 6)

    @pl.loop(0, nblk)
    def _(i):
        qkv_wait(i)

        @pl.when(i + 2 < nblk)
        def _():
            qkv_start(i + 2)

        def repack_job(n, j, r):
            def run(zero):
                even = wqkv_v[i * PPI + j, n, 0, r:r + 8, :] | zero
                odd = wqkv_v[i * PPI + j, n, 1, r:r + 8, :] | zero
                wqkv_v[i * PPI + j, n, 0, r:r + 8, :] = (even & _LO) | (odd << 16)
                wqkv_v[i * PPI + j, n, 1, r:r + 8, :] = (even >> 16) | (odd & _HI)
            return run

        jobs = [repack_job(n, j, r)
                for n in range(3) for j in range(PPI) for r in range(0, D // 2, 8)]
        per = -(-len(jobs) // (2 * nch))

        ra = pl.ds(pl.multiple_of(i * R, SB), SB)
        rb = pl.ds(pl.multiple_of(i * R + SB, SB), SB)
        la = la_v[pl.ds(pl.multiple_of(i * SB, SB), SB), :]
        xa, xb = g_v[ra, :], g_v[rb, :]
        lb = _layernorm(xb)
        h = D // 2
        lhs = _strassen_lhs(la[:, :h], la[:, h:], lb[:, :h], lb[:, h:])
        ms = [[None] * 7 for _ in range(nch)]
        for n in order[:2]:
            for c in range(2):
                ms[c][n] = _mm(lhs[n], _strassen_rhs(w3_v, t3_v, c, n))
        vs = []
        for c in range(nch):
            for n in order:
                if ms[c][n] is None:
                    ms[c][n] = _mm(lhs[n], _strassen_rhs(w3_v, t3_v, c, n))
            ua, ub = _strassen_out(ms[c])
            _spread(jobs, per, ua)
            _spread(jobs, per, ub)
            va, vb = _gelu(ua), _gelu(ub)
            vs.append(_strassen_lhs(va[:, :FC // 2], va[:, FC // 2:], vb[:, :FC // 2], vb[:, FC // 2:]))
        assert not jobs
        m = [None] * 7
        for n in order:
            m[n] = _mm(jnp.concatenate([v[n] for v in vs], axis=1),
                       jnp.concatenate([_strassen_rhs(w4_v, t4_v, c, n) for c in range(nch)], axis=0))
        ya, yb = _strassen_out(m)
        g_v[ra, h:] = _silu(xa[:, h:] + ya[:, h:])
        g_v[rb, :h] = _silu(xb[:, :h] + yb[:, :h])
        g_v[rb, h:] = _silu(xb[:, h:] + yb[:, h:])
        g_v[ra, :h] = _silu(xa[:, :h] + ya[:, :h])

    for c in a_copies:
        c.wait()

    row = lax.broadcasted_iota(jnp.int32, (L, L), 0)
    col = lax.broadcasted_iota(jnp.int32, (L, L), 1)
    mask = (row < M) | (row >= col)
    scale = Dh ** -0.5
    lag = 4
    bounds = tuple(k * H // (2 * lag) for k in range(lag + 1)) + (H,)

    def segment(s, mem):
        rows = pl.ds(pl.multiple_of(s * SEG, SEG), SEG)

        def project(h):
            w = jnp.concatenate([wqkv_v[h // 2, n, h % 2] for n in (1, 0, 2)], axis=1)
            return _mm(jnp.concatenate([mem, xn_v[rows, :]], axis=0), _w(w))

        def attend(kqv, sc):
            sc = jnp.where(mask, sc * scale, -1e9)
            p = jnp.exp(sc - jnp.max(sc, axis=-1, keepdims=True))
            den = jnp.sum(p, axis=-1, keepdims=True)
            r = pltpu.reciprocal(den, approx=True)
            r = r * (2.0 - den * r)
            return _mm(p * r, kqv[:, 2 * Dh:])

        def out_proj(h0, h1):
            o = jnp.concatenate([heads[h] for h in range(h0, h1)], axis=1)
            return _mm(o, _w(wo_v[h0 * Dh // 2:h1 * Dh // 2, :]))

        kqv, sc, heads, acc = {}, {}, {}, None
        for t in range(H + lag):
            if t < H:
                kqv[t] = project(t)
            else:
                y = out_proj(bounds[t - H], bounds[t - H + 1])
                acc = y if acc is None else acc + y
            if t >= lag:
                heads[t - lag] = attend(kqv.pop(t - lag), sc.pop(t - lag))
            if 1 <= t <= H:
                sc[t - 1] = _mm_nt(kqv[t - 1][:, Dh:2 * Dh], kqv[t - 1][:, :Dh])
        acc = acc + out_proj(bounds[-2], H)
        x_v[rows, :] = (x_v[rows, :].astype(F32) + acc[M:] * g_v[rows, :]).astype(BF16)
        return acc[:M]

    def step(i, mem):
        n = _SCAN_UNROLL
        for u in range(n):
            mem = segment(i * n + u, mem)
        rows = pl.ds(pl.multiple_of(i * n * SEG, n * SEG), n * SEG)
        pltpu.make_async_copy(x_v.at[rows, :], o_hbm.at[rows, :], sem_o.at[0]).start()
        return mem

    lax.fori_loop(0, S // SEG // _SCAN_UNROLL, step, mem0_v[...].astype(F32))
    pltpu.make_async_copy(x_v, o_hbm, sem_o.at[0]).wait()


@functools.partial(jax.jit, static_argnames=("A_seg_len",))
def pallas_recurrent_scan__memory_aug_recurrent_mem_tr__mixer_s_mlp__prompt_kernel(
    A_x: jax.Array,
    A_mem0: jax.Array,
    A_Wq: jax.Array,
    A_Wk: jax.Array,
    A_Wv: jax.Array,
    A_Wo: jax.Array,
    A_seg_len: int,
    B_x: jax.Array,
    B_w1: jax.Array,
    B_w2: jax.Array,
    B_w3: jax.Array,
    B_w4: jax.Array,
):
    del B_x
    B, S, D = A_x.shape
    _, H, Dh = A_Wq.shape
    M = A_mem0.shape[1]
    F = B_w3.shape[1]
    SEG = int(A_seg_len)
    nblk, nch = S // (2 * _SB), F // _FC
    assert B == 1 and S % (2 * _SB * _MIX_UNROLL) == 0 and S % (SEG * _SCAN_UNROLL) == 0
    assert F % _FC == 0 and nch <= nblk and (H // 2) % nblk == 0

    kern = functools.partial(_kernel, S=S, D=D, F=F, H=H, Dh=Dh, M=M, SEG=SEG)
    hbm = pl.BlockSpec(memory_space=pl.ANY)
    qkv_shape = (D // 2, 2, H, Dh)
    out = pl.pallas_call(
        kern,
        out_shape=jax.ShapeDtypeStruct((S, D), BF16),
        in_specs=[hbm] * 10,
        out_specs=hbm,
        scratch_shapes=[
            pltpu.VMEM((S, D), BF16),
            pltpu.VMEM((M, D), BF16),
            pltpu.VMEM((S, D), F32),
            pltpu.VMEM((_SB, D), BF16),
            pltpu.VMEM((S + 2 * _HALO, D), F32),
            pltpu.VMEM((S, D), F32),
            pltpu.VMEM((S // 2, D), F32),
            pltpu.VMEM((H // 2, 3, 2, D // 2, Dh), U32),
            pltpu.VMEM((H * Dh // 2, D), U32),
            pltpu.VMEM((D // 2, D), U32),
            pltpu.VMEM((1, D // 2, D), U32),
            pltpu.VMEM((nch, D // 2, _FC), U32),
            pltpu.VMEM((nch, _FC // 2, D), U32),
            pltpu.VMEM((1, 5, D // 4, D // 2), U32),
            pltpu.VMEM((nch, 5, D // 4, _FC // 2), U32),
            pltpu.VMEM((nch, 5, _FC // 4, D // 2), U32),
            pltpu.SemaphoreType.DMA((_NC + 8,)),
            pltpu.SemaphoreType.DMA((2 * nch,)),
            pltpu.SemaphoreType.DMA((nblk,)),
            pltpu.SemaphoreType.DMA((1,)),
        ],
        compiler_params=pltpu.CompilerParams(
            vmem_limit_bytes=120 * 1024 * 1024, disable_bounds_checks=True),
        name="rmt_mixer",
    )(
        A_x.reshape(S, D),
        A_mem0.reshape(M, D),
        A_Wq.reshape(qkv_shape),
        A_Wk.reshape(qkv_shape),
        A_Wv.reshape(qkv_shape),
        A_Wo.reshape(H * Dh, D),
        B_w1, B_w2, B_w3, B_w4,
    )
    return out.reshape(B, S, D)
```

```python
import functools

import jax
import jax.numpy as jnp
import numpy as np
from jax import lax
from jax.experimental import pallas as pl
from jax.experimental.pallas import tpu as pltpu

F32 = jnp.float32
BF16 = jnp.bfloat16
U32 = jnp.uint32
_LO = np.uint32(0x0000FFFF)
_HI = np.uint32(0xFFFF0000)
_EPS = 1e-5
_HALO = 8
_SB = 128
_FC = 512
_NC = 4
_MIX_UNROLL = 2
_SCAN_UNROLL = 2


def _mm(a, b):
    return lax.dot_general(a, b, (((1,), (0,)), ((), ())), preferred_element_type=F32)


def _mm_nt(a, b):
    return lax.dot_general(a, b, (((1,), (1,)), ((), ())), preferred_element_type=F32)


def _w(u):
    return pltpu.bitcast(u, BF16)


def _layernorm(x):
    m = jnp.mean(x, axis=-1, keepdims=True)
    d = x - m
    v = jnp.mean(d * d, axis=-1, keepdims=True)
    return d * lax.rsqrt(v + _EPS)


def _gelu(x):
    c = float(np.sqrt(2.0 / np.pi))
    t = jnp.tanh(x * (c + (c * 0.044715) * (x * x)))
    hx = 0.5 * x
    return hx + hx * t


def _silu(x):
    hx = 0.5 * x
    return hx + hx * jnp.tanh(hx)


def _strassen_lhs(a11, a12, a21, a22):
    ops = (a11 + a22, a21 + a22, a11, a22, a11 + a12, a21 - a11, a12 - a22)
    return [o.astype(BF16) for o in ops]


def _strassen_rhs(w_v, t_v, c, n):
    kh, nh = w_v.shape[1] // 2, w_v.shape[2] // 2
    if n == 1:
        return _w(w_v[c, :kh, :nh])
    if n == 4:
        return _w(w_v[c, kh:, nh:])
    return t_v[c, {0: 0, 2: 1, 3: 2, 5: 3, 6: 4}[n]]


def _strassen_out(m):
    top = jnp.concatenate([m[0] + m[3] - m[4] + m[6], m[2] + m[4]], axis=1)
    bot = jnp.concatenate([m[1] + m[3], m[0] - m[1] + m[2] + m[5]], axis=1)
    return top, bot


def _presum_jobs(w_v, t_v, g0, ng, l0=0, l1=None):
    kh, nh = w_v.shape[1] // 2, w_v.shape[2] // 2

    def job(g, l):
        def run(zero):
            c, r = g // (kh // 8), g % (kh // 8) * 8
            r2 = 2 * r
            if not isinstance(r, int):
                r, r2 = pl.multiple_of(r, 8), pl.multiple_of(r2, 16)

            def quad(i, j):
                u = w_v[c, pl.ds(i * kh + r, 8), j * nh + l:j * nh + l + 256]
                if zero is not None and i == j:
                    u = u | jnp.concatenate([zero, zero], axis=1)
                return _w(u).astype(F32)

            b11, b12, b21, b22 = quad(0, 0), quad(0, 1), quad(1, 0), quad(1, 1)
            for n, t in enumerate((b11 + b22, b12 - b22, b21 - b11, b11 + b12, b21 + b22)):
                t_v[c, n, pl.ds(r2, 16), l:l + 256] = t.astype(BF16)
        return run

    return [job(g0 + g, l) for g in range(ng) for l in range(l0, nh if l1 is None else l1, 256)]


def _spread(jobs, n, after):
    tiles = [(r, c) for c in range(0, after.shape[1], 128) for r in range(0, after.shape[0], 8)]
    n = min(n, len(jobs))
    for k in range(n):
        r, c = tiles[k * len(tiles) // n]
        zero = lax.population_count(pltpu.bitcast(after[r:r + 8, c:c + 128], U32)) >> 6
        jobs.pop(0)(zero)


def _kernel(x_hbm, mem0_hbm, wq_hbm, wk_hbm, wv_hbm, wo_hbm, w1_hbm, w2_hbm, w3_hbm, w4_hbm,
            o_hbm,
            x_v, mem0_v, xn_v, p_v, hb_v, g_v, la_v,
            wqkv_v, wo_v, w1_v, w2_v, w3_v, w4_v, t1_v, t2_v, t3_v, t4_v,
            sem_w, sem_m, sem_a, sem_o,
            *, S, D, F, H, Dh, M, SEG):
    SB, FC, NC = _SB, _FC, _NC
    R = 2 * SB
    nblk = S // R
    nsb = S // SB
    nch = F // FC
    L = M + SEG
    PPI = H // 2 // nblk
    CW = D // NC

    sems = iter(range(sem_w.shape[0]))

    def copy(src, dst):
        return pltpu.make_async_copy(src, dst, sem_w.at[next(sems)])

    x_copies = [copy(x_hbm.at[lo * SB:hi * SB, :], x_v.at[lo * SB:hi * SB, :])
                for lo, hi in ((0, 2), (2, 3), (3, 5), (5, 7), (7, nsb))]
    w1u, w3u, w4u = w1_hbm.bitcast(U32), w3_hbm.bitcast(U32), w4_hbm.bitcast(U32)
    w1_copies = [copy(w1u.at[:, c * CW:(c + 1) * CW], w1_v.at[0, :, c * CW:(c + 1) * CW])
                 for c in range(NC)]
    w2_copy = copy(w2_hbm.bitcast(U32), w2_v.at[0])
    a_copies = [copy(mem0_hbm, mem0_v), copy(wo_hbm.bitcast(U32), wo_v)]

    def mlp_copies(c):
        return [pltpu.make_async_copy(w3u.at[:, pl.ds(c * FC, FC)], w3_v.at[c], sem_m.at[c]),
                pltpu.make_async_copy(w4u.at[pl.ds(c * (FC // 2), FC // 2), :], w4_v.at[c],
                                      sem_m.at[nch + c])]

    def qkv_start(i):
        for n, src in enumerate((wq_hbm, wk_hbm, wv_hbm)):
            for j in range(PPI):
                for p in range(2):
                    pltpu.make_async_copy(src.bitcast(U32).at[:, p, i * PPI + j, :],
                                          wqkv_v.at[i * PPI + j, n, p], sem_a.at[i]).start()

    def qkv_wait(i):
        dst = wqkv_v.at[pl.ds(i * PPI, PPI)]
        pltpu.make_async_copy(dst, dst, sem_a.at[i]).wait()

    for c in (x_copies[:1] + w1_copies[:-1] + x_copies[1:2] + w1_copies[-1:] + x_copies[2:]
              + [w2_copy]):
        c.start()
    for c in range(nch):
        for cp in mlp_copies(c):
            cp.start()

    for t in range(D // 128):
        hb_v[t, 0:_HALO, :] = jnp.zeros((_HALO, 128), F32)
        hb_v[t, _HALO + S:, :] = jnp.zeros((_HALO, 128), F32)
    h = D // 2
    order = (2, 4, 3, 1, 0, 5, 6)

    def norm(r0):
        xn = _layernorm(x_v[pl.ds(r0, SB), :].astype(F32))
        xn_v[pl.ds(r0, SB), :] = xn
        return _layernorm(xn)

    def put_hidden(r0, c0, y):
        y = _gelu(y)
        for c in range(0, y.shape[1], 128):
            hb_v[(c0 + c) // 128, pl.ds(r0 + _HALO, SB), :] = y[:, c:c + 128]

    x_copies[0].wait()
    xnn = [norm(0).astype(BF16), norm(SB).astype(BF16)]
    for n in range(NC):
        if n == NC - 1:
            x_copies[1].wait()
        w1_copies[n].wait()
        l0 = (n - NC // 2) * CW
        jobs = _presum_jobs(w1_v, t1_v, 0, D // 32, l0, l0 + CW) if l0 >= 0 else []
        per = len(jobs) // 2
        for b in range(2):
            y = _mm(xnn[b], _w(w1_v[0, :, n * CW:(n + 1) * CW]))
            _spread(jobs, per, y)
            put_hidden(b * SB, n * CW, y)
        assert not jobs
    p_v[...] = norm(2 * SB)

    @pl.loop(1, nblk)
    def _(i):
        for k in range(1, 4):
            @pl.when(i == k)
            def _():
                x_copies[k + 1].wait()
        r0 = pl.multiple_of(i * R, SB)
        a, b = p_v[...], norm(r0 + SB)
        lhs = _strassen_lhs(a[:, :h], a[:, h:], b[:, :h], b[:, h:])
        m = [None] * 7
        for k, n in enumerate(order):
            if k == 1:
                p_v[...] = norm(pl.multiple_of(jnp.minimum(r0 + R, S - SB), SB))
            m[n] = _mm(lhs[n], _strassen_rhs(w1_v, t1_v, 0, n))
        top, bot = _strassen_out(m)
        put_hidden(r0, h, top[:, h:])
        put_hidden(r0 + SB, 0, bot[:, :h])
        put_hidden(r0 + SB, h, bot[:, h:])
        put_hidden(r0, 0, top[:, :h])

    w2_copy.wait()
    qkv_start(0)
    qkv_start(1)
    for job in _presum_jobs(w2_v, t2_v, 0, D // 32):
        job(None)

    def shifted(r0):
        shifts = (-1, 1, -2, 2)
        return jnp.concatenate(
            [hb_v[t, pl.ds(r0 + _HALO + shifts[t * 128 // (D // 4)], SB), :]
             for t in range(D // 128)], axis=1)

    @pl.loop(0, nblk // _MIX_UNROLL)
    def _(it):
        blocks = [it * _MIX_UNROLL + u for u in range(_MIX_UNROLL)]
        for i in blocks:
            @pl.when(i < nch)
            def _():
                for cp in mlp_copies(i):
                    cp.wait()
        g3 = nch * (D // 32) * _MIX_UNROLL // nblk
        g4 = nch * (FC // 32) * _MIX_UNROLL // nblk
        jobs = _presum_jobs(w3_v, t3_v, it * g3, g3) + _presum_jobs(w4_v, t4_v, it * g4, g4)
        per = -(-len(jobs) // (7 * _MIX_UNROLL))
        for i in blocks:
            r0 = [pl.multiple_of(i * R + b * SB, SB) for b in range(2)]
            ha, hb = shifted(r0[0]), shifted(r0[1])
            lhs = _strassen_lhs(ha[:, :h], ha[:, h:], hb[:, :h], hb[:, h:])
            m = [None] * 7
            for n in (2, 4, 3, 0, 6, 1, 5):
                m[n] = _mm(lhs[n], _strassen_rhs(w2_v, t2_v, 0, n))
                _spread(jobs, per, m[n])
            hs = _strassen_out(m)
            xs = [xn_v[pl.ds(r, SB), :] for r in r0]
            for b in range(2):
                x1 = xs[b] + hs[b]
                g_v[pl.ds(r0[b], SB), :] = x1
                if b == 0:
                    la_v[pl.ds(pl.multiple_of(i * SB, SB), SB), :] = _layernorm(x1)
        assert not jobs

    for c in a_copies:
        c.start()

    @pl.loop(0, nblk)
    def _(i):
        qkv_wait(i)

        @pl.when(i + 2 < nblk)
        def _():
            qkv_start(i + 2)

        def repack_job(n, j, r):
            def run(zero):
                even = wqkv_v[i * PPI + j, n, 0, r:r + 8, :] | zero
                odd = wqkv_v[i * PPI + j, n, 1, r:r + 8, :] | zero
                wqkv_v[i * PPI + j, n, 0, r:r + 8, :] = (even & _LO) | (odd << 16)
                wqkv_v[i * PPI + j, n, 1, r:r + 8, :] = (even >> 16) | (odd & _HI)
            return run

        jobs = [repack_job(n, j, r)
                for n in range(3) for j in range(PPI) for r in range(0, D // 2, 8)]
        per = -(-len(jobs) // (2 * nch))

        ra = pl.ds(pl.multiple_of(i * R, SB), SB)
        rb = pl.ds(pl.multiple_of(i * R + SB, SB), SB)
        la = la_v[pl.ds(pl.multiple_of(i * SB, SB), SB), :]
        xa, xb = g_v[ra, :], g_v[rb, :]
        lb = _layernorm(xb)
        lhs = _strassen_lhs(la[:, :h], la[:, h:], lb[:, :h], lb[:, h:])
        ms = [[None] * 7 for _ in range(nch)]
        for n in order[:2]:
            for c in range(2):
                ms[c][n] = _mm(lhs[n], _strassen_rhs(w3_v, t3_v, c, n))
        vs = []
        for c in range(nch):
            for n in order:
                if ms[c][n] is None:
                    ms[c][n] = _mm(lhs[n], _strassen_rhs(w3_v, t3_v, c, n))
            ua, ub = _strassen_out(ms[c])
            _spread(jobs, per, ua)
            _spread(jobs, per, ub)
            va, vb = _gelu(ua), _gelu(ub)
            vs.append(_strassen_lhs(va[:, :FC // 2], va[:, FC // 2:], vb[:, :FC // 2], vb[:, FC // 2:]))
        assert not jobs
        m = [None] * 7
        for n in order:
            m[n] = _mm(jnp.concatenate([v[n] for v in vs], axis=1),
                       jnp.concatenate([_strassen_rhs(w4_v, t4_v, c, n) for c in range(nch)], axis=0))
        ya, yb = _strassen_out(m)
        g_v[ra, h:] = _silu(xa[:, h:] + ya[:, h:])
        g_v[rb, :h] = _silu(xb[:, :h] + yb[:, :h])
        g_v[rb, h:] = _silu(xb[:, h:] + yb[:, h:])
        g_v[ra, :h] = _silu(xa[:, :h] + ya[:, :h])

    for c in a_copies:
        c.wait()

    row = lax.broadcasted_iota(jnp.int32, (L, L), 0)
    col = lax.broadcasted_iota(jnp.int32, (L, L), 1)
    mask = (row < M) | (row >= col)
    scale = Dh ** -0.5
    lag = 4
    bounds = tuple(k * H // (2 * lag) for k in range(lag + 1)) + (H,)

    def segment(s, mem):
        rows = pl.ds(pl.multiple_of(s * SEG, SEG), SEG)

        def project(hd):
            w = jnp.concatenate([wqkv_v[hd // 2, n, hd % 2] for n in (1, 0, 2)], axis=1)
            return _mm(jnp.concatenate([mem, xn_v[rows, :]], axis=0), _w(w))

        def attend(kqv, sc):
            sc = jnp.where(mask, sc * scale, -1e9)
            p = jnp.exp(sc - jnp.max(sc, axis=-1, keepdims=True))
            den = jnp.sum(p, axis=-1, keepdims=True)
            r = pltpu.reciprocal(den, approx=True)
            r = r * (2.0 - den * r)
            return _mm(p * r, kqv[:, 2 * Dh:])

        def out_proj(h0, h1):
            o = jnp.concatenate([heads[hd] for hd in range(h0, h1)], axis=1)
            return _mm(o, _w(wo_v[h0 * Dh // 2:h1 * Dh // 2, :]))

        kqv, sc, heads, acc = {}, {}, {}, None
        for t in range(H + lag):
            if t < H:
                kqv[t] = project(t)
            else:
                y = out_proj(bounds[t - H], bounds[t - H + 1])
                acc = y if acc is None else acc + y
            if t >= lag:
                heads[t - lag] = attend(kqv.pop(t - lag), sc.pop(t - lag))
            if 1 <= t <= H:
                sc[t - 1] = _mm_nt(kqv[t - 1][:, Dh:2 * Dh], kqv[t - 1][:, :Dh])
        acc = acc + out_proj(bounds[-2], H)
        x_v[rows, :] = (x_v[rows, :].astype(F32) + acc[M:] * g_v[rows, :]).astype(BF16)
        return acc[:M]

    def step(i, mem):
        n = _SCAN_UNROLL
        for u in range(n):
            mem = segment(i * n + u, mem)
        rows = pl.ds(pl.multiple_of(i * n * SEG, n * SEG), n * SEG)
        pltpu.make_async_copy(x_v.at[rows, :], o_hbm.at[rows, :], sem_o.at[0]).start()
        return mem

    lax.fori_loop(0, S // SEG // _SCAN_UNROLL, step, mem0_v[...].astype(F32))
    pltpu.make_async_copy(x_v, o_hbm, sem_o.at[0]).wait()


@functools.partial(jax.jit, static_argnames=("A_seg_len",))
def pallas_recurrent_scan__memory_aug_recurrent_mem_tr__mixer_s_mlp__prompt_kernel(
    A_x: jax.Array,
    A_mem0: jax.Array,
    A_Wq: jax.Array,
    A_Wk: jax.Array,
    A_Wv: jax.Array,
    A_Wo: jax.Array,
    A_seg_len: int,
    B_x: jax.Array,
    B_w1: jax.Array,
    B_w2: jax.Array,
    B_w3: jax.Array,
    B_w4: jax.Array,
):
    del B_x
    B, S, D = A_x.shape
    _, H, Dh = A_Wq.shape
    M = A_mem0.shape[1]
    F = B_w3.shape[1]
    SEG = int(A_seg_len)
    nblk, nch = S // (2 * _SB), F // _FC
    assert B == 1 and S % (2 * _SB * _MIX_UNROLL) == 0 and S % (SEG * _SCAN_UNROLL) == 0
    assert F % _FC == 0 and nch <= nblk and (H // 2) % nblk == 0
    assert nch * (_FC // 32) * _MIX_UNROLL % nblk == 0 and D // _NC == 256

    kern = functools.partial(_kernel, S=S, D=D, F=F, H=H, Dh=Dh, M=M, SEG=SEG)
    hbm = pl.BlockSpec(memory_space=pl.ANY)
    qkv_shape = (D // 2, 2, H, Dh)
    out = pl.pallas_call(
        kern,
        out_shape=jax.ShapeDtypeStruct((S, D), BF16),
        in_specs=[hbm] * 10,
        out_specs=hbm,
        scratch_shapes=[
            pltpu.VMEM((S, D), BF16),
            pltpu.VMEM((M, D), BF16),
            pltpu.VMEM((S, D), F32),
            pltpu.VMEM((_SB, D), F32),
            pltpu.VMEM((D // 128, S + 2 * _HALO, 128), F32),
            pltpu.VMEM((S, D), F32),
            pltpu.VMEM((S // 2, D), F32),
            pltpu.VMEM((H // 2, 3, 2, D // 2, Dh), U32),
            pltpu.VMEM((H * Dh // 2, D), U32),
            pltpu.VMEM((1, D // 2, D), U32),
            pltpu.VMEM((1, D // 2, D), U32),
            pltpu.VMEM((nch, D // 2, _FC), U32),
            pltpu.VMEM((nch, _FC // 2, D), U32),
            pltpu.VMEM((1, 5, D // 2, D // 2), BF16),
            pltpu.VMEM((1, 5, D // 2, D // 2), BF16),
            pltpu.VMEM((nch, 5, D // 2, _FC // 2), BF16),
            pltpu.VMEM((nch, 5, _FC // 2, D // 2), BF16),
            pltpu.SemaphoreType.DMA((_NC + 8,)),
            pltpu.SemaphoreType.DMA((2 * nch,)),
            pltpu.SemaphoreType.DMA((nblk,)),
            pltpu.SemaphoreType.DMA((1,)),
        ],
        compiler_params=pltpu.CompilerParams(
            vmem_limit_bytes=120 * 1024 * 1024, disable_bounds_checks=True),
        name="rmt_mixer",
    )(
        A_x.reshape(S, D),
        A_mem0.reshape(M, D),
        A_Wq.reshape(qkv_shape),
        A_Wk.reshape(qkv_shape),
        A_Wv.reshape(qkv_shape),
        A_Wo.reshape(H * Dh, D),
        B_w1, B_w2, B_w3, B_w4,
    )
    return out.reshape(B, S, D)
```
